```python
import os as _os
_os.environ.setdefault("JAX_PLATFORMS", "cpu")
import jax
import jax.numpy as jnp

def _softmax(x, axis=-1):
    return jax.nn.softmax(x, axis=axis)
def _gelu(x):
    return jax.nn.gelu(x, approximate=True)
def _silu(x):
    return jax.nn.silu(x)
def _sigmoid(x):
    return jax.nn.sigmoid(x)
def _layernorm(x, axis=-1, eps=1e-5):
    m = jnp.mean(x, axis=axis, keepdims=True)
    v = jnp.var(x, axis=axis, keepdims=True)
    return (x - m) / jnp.sqrt(v + eps)
def _scatter_add(tgt, idx, src, axis=0):
    return tgt.at[idx].add(src)
def _segment_sum(src, seg, n):
    return jax.ops.segment_sum(src, seg, n)
class _Rng:
    def __init__(self, key):
        self._k = key
    def _next(self):
        self._k, sub = jax.random.split(self._k)
        return sub
    def normal(self, shape):
        return jax.random.normal(self._next(), shape, dtype=jnp.bfloat16)
    def randint(self, lo, hi, shape):
        return jax.random.randint(self._next(), shape, lo, hi, dtype=jnp.int32)
    def uniform(self, shape, lo=0.0, hi=1.0):
        return jax.random.uniform(self._next(), shape, jnp.bfloat16, lo, hi)
    def permutation(self, n):
        return jax.random.permutation(self._next(), n)


kernel_name = 'sequential_preLN__linear_attn_block__glu_gated_reglu__prompt'

def setup_inputs():
    _rng = _Rng(jax.random.key(int.from_bytes(__import__("os").urandom(4), "little")))
    _w = (lambda a: (lambda t: t.astype(jnp.bfloat16) if jnp.issubdtype(t.dtype, jnp.floating) else t)(jnp.asarray(a)))
    def _A_setup():
        B, S, D = 1, 2048, 640
        return {
            "x": _w((lambda *s: _rng.normal(s) * 0.05)(B, S, D)),
            "wqkv": _w((lambda *s: _rng.normal(s) * 0.05)(D, 3 * D)),
            "wo": _w((lambda *s: _rng.normal(s) * 0.05)(D, D)),
        }
    _A_in = _A_setup()

    def _B_setup():
        B, S, D, F = 1, 2048, 640, 1536
        return {
            "x": _w((lambda *s: _rng.normal(s) * 0.05)(B, S, D)),
            "W_gate": _w((lambda *s: _rng.normal(s) * 0.05)(D, F) * (2.0 / D) ** 0.5),
            "W_up": _w((lambda *s: _rng.normal(s) * 0.05)(D, F) * (2.0 / D) ** 0.5),
            "W_down": _w((lambda *s: _rng.normal(s) * 0.05)(F, D) * (1.0 / F) ** 0.5),
        }
    _B_in = _B_setup()

    return {
        "A_x": _A_in["x"],
        "A_wqkv": _A_in["wqkv"],
        "A_wo": _A_in["wo"],
        "B_x": _B_in["x"],
        "B_W_gate": _B_in["W_gate"],
        "B_W_up": _B_in["W_up"],
        "B_W_down": _B_in["W_down"],
    }

def reference(A_x, A_wqkv, A_wo, B_x, B_W_gate, B_W_up, B_W_down):
    def _A_ref(x, wqkv, wo):
        B, S, D = x.shape
        H = 32; Dh = D // H
        qkv = (lambda x, *d: x.transpose(*d))((x @ wqkv).reshape(B, S, 3, H, Dh), 2, 0, 3, 1, 4)
        q, k, v = qkv[0], qkv[1], qkv[2]
        phi = lambda t: jnp.where(t > 0, t + 1, jnp.exp(t)) + 1e-6
        pq, pk = phi(q), phi(k)
        kv = jnp.einsum("bhsd,bhse->bhde", pk, v)
        z = jnp.einsum("bhsd->bhd", pk)
        num = jnp.einsum("bhqd,bhde->bhqe", pq, kv)
        den = jnp.einsum("bhqd,bhd->bhq", pq, z)[..., None] + 1e-6
        o = num / den
        return (lambda x, *d: x.transpose(*d))(o, 0, 2, 1, 3).reshape(B, S, D) @ wo

    def _B_ref(x, W_gate, W_up, W_down):
        gate = jnp.einsum("bsd,df->bsf", x, W_gate)
        up = jnp.einsum("bsd,df->bsf", x, W_up)
        gate = gate * (lambda x, dt: x.astype(dt))(gate > 0, gate.dtype)
        h = gate * up
        return jnp.einsum("bsf,fd->bsd", h, W_down)

    x = A_x
    h = x + _A_ref(_layernorm(x, axis=-1), A_wqkv, A_wo)
    h2 = h + _B_ref(_layernorm(h, axis=-1), B_W_gate, B_W_up, B_W_down)
    return h2
```

```python
import functools
import jax
import jax.numpy as jnp
from jax import lax
import jax.experimental.pallas as pl
import jax.experimental.pallas.tpu as pltpu

S, D, F, H, DH = 2048, 640, 1536, 32, 20
TM0 = 256
NB0 = S // TM0
TM1 = 512
NB1 = S // TM1
NT = D // 128
NSPLIT_LAST = 2
f32 = jnp.float32
bf16 = jnp.bfloat16
BAND = [(0, 144), (120, 264), (240, 400), (376, 520), (496, 640)]


def _ln(x):
    m = jnp.mean(x, axis=-1, keepdims=True)
    xc = x - m
    v = jnp.mean(xc * xc, axis=-1, keepdims=True)
    return xc * lax.rsqrt(v + 1e-5)


def _phi(t):
    return jnp.where(t > 0, t + 1.0, jnp.exp(t)) + 1e-6


def _dot(a, b):
    return jnp.dot(a, b, preferred_element_type=f32)


def _kernel(x_hbm, wqkv_hbm, wo_hbm, wg_hbm, wu_hbm, wd_hbm, o_hbm,
            x_v, wq_v, wk_v, wv_v, wo_v, wg_v, wu_v, wd_v, wqp_v,
            ln_v, g_v, macc_v, m_v, zp_v, t_v, t2_v, pq_v, h_v, ln2_v, o_v,
            sem_x, sem_w, sem_o):
    xr = [(0, TM0), (TM0, 3 * TM0), (3 * TM0, 5 * TM0), (5 * TM0, S)]
    xcopies = [pltpu.make_async_copy(x_hbm.at[lo:hi, :], x_v.at[lo:hi, :], sem_x.at[j])
               for j, (lo, hi) in enumerate(xr)]
    wcopies = [
        pltpu.make_async_copy(wqkv_hbm.at[:, D:2 * D], wk_v, sem_w.at[0]),
        pltpu.make_async_copy(wqkv_hbm.at[:, 0:D], wq_v, sem_w.at[1]),
        pltpu.make_async_copy(wqkv_hbm.at[:, 2 * D:3 * D], wv_v, sem_w.at[2]),
        pltpu.make_async_copy(wo_hbm, wo_v, sem_w.at[3]),
        pltpu.make_async_copy(wg_hbm, wg_v, sem_w.at[4]),
        pltpu.make_async_copy(wu_hbm, wu_v, sem_w.at[5]),
        pltpu.make_async_copy(wd_hbm, wd_v, sem_w.at[6]),
    ]

    def ocopy(r0, n, j):
        return pltpu.make_async_copy(o_v.at[pl.ds(r0, n), :],
                                     o_hbm.at[pl.ds(r0, n), :], sem_o.at[j])

    def perm_lanes(a, tref):
        tref[...] = a.T
        parts = [tref[pl.ds(d, H, stride=DH), :] for d in range(DH)]
        return jnp.concatenate(parts, axis=0).T

    def ln1(i):
        sl = slice(i * TM0, (i + 1) * TM0)
        ln_v[sl, :] = _ln(x_v[sl, :].astype(f32)).astype(bf16)

    def kdot(i):
        return _dot(ln_v[i * TM0:(i + 1) * TM0, :], wk_v[...])

    xcopies[0].start()
    wcopies[0].start()
    macc_v[...] = jnp.zeros_like(macc_v)
    xcopies[0].wait()
    xcopies[1].start()
    ln1(0)
    wcopies[0].wait()
    xcopies[2].start()
    k = kdot(0)
    xcopies[1].wait()
    xcopies[3].start()
    wcopies[1].start()
    ln1(1)

    z = None
    for i in range(NB0):
        if i == 1:
            xcopies[2].wait()
            wcopies[2].start()
            wcopies[3].start()
        if i == 3:
            xcopies[3].wait()
            wcopies[1].wait()
            for c in wcopies[4:]:
                c.start()
        if i + 2 < NB0:
            ln1(i + 2)
        if i + 1 < NB0:
            k_next = kdot(i + 1)
        pk = _phi(k)
        zi = jnp.sum(pk, axis=0, keepdims=True)
        z = zi if z is None else z + zi
        gi = lax.dot_general(pk.astype(bf16), ln_v[i * TM0:(i + 1) * TM0, :],
                             (((0,), (0,)), ((), ())), preferred_element_type=f32)
        if i == 0:
            g_v[...] = gi
        else:
            g_v[...] += gi
        if 3 <= i < 3 + NT:
            c0 = (i - 3) * 128
            wqp_v[c0:c0 + 128, :] = perm_lanes(
                wq_v[c0:c0 + 128, :].astype(f32), t_v).astype(bf16)
        k = k_next

    wcopies[2].wait()
    wcopies[3].wait()

    def qdot(i):
        sl = slice(i * TM1, (i + 1) * TM1)
        pq_v[sl, :] = _phi(_dot(ln_v[sl, :], wqp_v[...]))

    zp_v[...] = perm_lanes(jnp.broadcast_to(z, (128, D)), t2_v)[0:8, :]
    qdot(0)
    kvs = []
    for b, (lo, hi) in enumerate(BAND):
        n = hi - lo
        kvb = _dot(g_v[lo:hi, :].astype(bf16), wv_v[:, 128 * b:128 * (b + 1)])
        rh = (lax.broadcasted_iota(jnp.int32, (n, 128), 0) + lo) // DH
        ch = (lax.broadcasted_iota(jnp.int32, (n, 128), 1) + 128 * b) // DH
        kvs.append(jnp.where(rh == ch, kvb, 0.0).astype(bf16))
    qdot(1)
    for b, (lo, hi) in enumerate(BAND):
        res = _dot(kvs[b], wo_v[128 * b:128 * (b + 1), :])
        for c in range(NT):
            macc_v[c, lo:hi, :] += res[:, 128 * c:128 * (c + 1)]
    qdot(2)
    for c in range(NT):
        for d in range(DH):
            m_v[H * d:H * (d + 1), 128 * c:128 * (c + 1)] = macc_v[
                c, pl.ds(d, H, stride=DH), :].astype(bf16)

    def norm(r0):
        pq = pq_v[pl.ds(r0, TM1), :]
        zp = zp_v[0:1, :]
        t = pq[:, 0:128] * zp[:, 0:128]
        for c in range(1, NT):
            t = t + pq[:, 128 * c:128 * (c + 1)] * zp[:, 128 * c:128 * (c + 1)]
        t = t + pltpu.roll(t, 64, 1)
        t = t + pltpu.roll(t, 32, 1)
        r = 1.0 / (t + 1e-6)
        return jnp.concatenate(
            [(pq[:, 128 * c:128 * (c + 1)] * r).astype(bf16) for c in range(NT)], axis=1)

    def attn(r0, pqn):
        h = x_v[pl.ds(r0, TM1), :].astype(f32) + _dot(pqn, m_v[...])
        h_v[pl.ds(r0, TM1), :] = h
        return h

    def ln2(r0, h):
        ln2_v[pl.ds(r0, TM1), :] = _ln(h).astype(bf16)

    def gateup(r0):
        l2 = ln2_v[pl.ds(r0, TM1), :]
        gate = _dot(l2, wg_v[...])
        up = _dot(l2, wu_v[...])
        return (jnp.maximum(gate, 0.0) * up).astype(bf16)

    h0 = attn(0, norm(0))
    for c in wcopies[4:]:
        c.wait()
    qdot(3)
    ln2(0, h0)

    def loop_1(i, c):
        r0 = i * TM1
        r1 = (i + 1) * TM1
        act = gateup(r0)
        h1 = attn(r1, norm(r1))
        out = h_v[pl.ds(r0, TM1), :] + _dot(act, wd_v[...])
        o_v[pl.ds(r0, TM1), :] = out.astype(bf16)
        ln2(r1, h1)
        ocopy(r0, TM1, i).start()
        return c

    for _i in range(NB1 - 1):
        loop_1(_i, 0)
    r0 = (NB1 - 1) * TM1
    act = gateup(r0)
    n = TM1 // NSPLIT_LAST
    for j in range(NSPLIT_LAST):
        rr = r0 + j * n
        out = h_v[rr:rr + n, :] + _dot(act[j * n:(j + 1) * n, :], wd_v[...])
        o_v[rr:rr + n, :] = out.astype(bf16)
        ocopy(rr, n, NB1 - 1 + j).start()
    for i in range(NB1 - 1):
        ocopy(i * TM1, TM1, i).wait()
    for j in range(NSPLIT_LAST):
        ocopy(r0 + j * n, n, NB1 - 1 + j).wait()


@jax.jit
def pallas_sequential_preLN__linear_attn_block__glu_gated_reglu__prompt_kernel(
    A_x, A_wqkv, A_wo, B_x, B_W_gate, B_W_up, B_W_down,
):
    x = A_x.reshape(S, D)
    anyspec = pl.BlockSpec(memory_space=pl.ANY)
    out = pl.pallas_call(
        _kernel,
        in_specs=[anyspec] * 6,
        out_specs=anyspec,
        out_shape=jax.ShapeDtypeStruct((S, D), bf16),
        scratch_shapes=[
            pltpu.VMEM((S, D), bf16),
            pltpu.VMEM((D, D), bf16),
            pltpu.VMEM((D, D), bf16),
            pltpu.VMEM((D, D), bf16),
            pltpu.VMEM((D, D), bf16),
            pltpu.VMEM((D, F), bf16),
            pltpu.VMEM((D, F), bf16),
            pltpu.VMEM((F, D), bf16),
            pltpu.VMEM((D, D), bf16),
            pltpu.VMEM((S, D), bf16),
            pltpu.VMEM((D, D), f32),
            pltpu.VMEM((NT, D, 128), f32),
            pltpu.VMEM((D, D), bf16),
            pltpu.VMEM((8, D), f32),
            pltpu.VMEM((D, 128), f32),
            pltpu.VMEM((D, 128), f32),
            pltpu.VMEM((S, D), f32),
            pltpu.VMEM((S, D), f32),
            pltpu.VMEM((S, D), bf16),
            pltpu.VMEM((S, D), bf16),
            pltpu.SemaphoreType.DMA((4,)),
            pltpu.SemaphoreType.DMA((7,)),
            pltpu.SemaphoreType.DMA((NB1 - 1 + NSPLIT_LAST,)),
        ],
        compiler_params=pltpu.CompilerParams(
            vmem_limit_bytes=100 * 1024 * 1024,
        ),
    )(x, A_wqkv, A_wo, B_W_gate, B_W_up, B_W_down)
    return out.reshape(1, S, D)
```

```python
import jax
import jax.numpy as jnp
from jax import lax
import jax.experimental.pallas as pl
import jax.experimental.pallas.tpu as pltpu

S, D, F, H, DH = 2048, 640, 1536, 32, 20
TM0 = 256
NB0 = S // TM0
TM1 = 256
TQ = 512
NB1 = S // TM1
NT = D // 128
TAILC = [(0, 512), (512, 640)]
CH = 32
KCH = [(0, 2), (2, 4), (4, 5)]
f32 = jnp.float32
bf16 = jnp.bfloat16
BAND = [(0, 144), (120, 264), (240, 400), (376, 520), (496, 640)]


def _ln(x):
    m = jnp.mean(x, axis=-1, keepdims=True)
    xc = x - m
    v = jnp.mean(xc * xc, axis=-1, keepdims=True)
    return xc * lax.rsqrt(v + 1e-5)


def _phi(t):
    return jnp.where(t > 0, t + 1.0, jnp.exp(t)) + 1e-6


def _dot(a, b):
    return jnp.dot(a, b, preferred_element_type=f32)


def _kernel(x_hbm, wqkv_hbm, wo_hbm, wg_hbm, wu_hbm, wd_hbm, o_hbm,
            x_v, wq_v, wk_v, wv_v, wo_v, wg_v, wu_v, wd_v, wqp_v,
            ln_v, g_v, macc_v, m_v, zp_v, t_v, t2_v, pq_v, pqn_v, h_v, ln2_v, o_v, act_v, z_s,
            sem_w, sem_o):
    xr = [(0, TM0), (TM0, 2 * TM0), (2 * TM0, 4 * TM0), (4 * TM0, S)]
    xcopies = [pltpu.make_async_copy(x_hbm.at[lo:hi, :], x_v.at[lo:hi, :], sem_w.at[6 + j])
               for j, (lo, hi) in enumerate(xr)]
    kcopies = [pltpu.make_async_copy(wqkv_hbm.at[:, D + 128 * c:D + 128 * (c + 1)],
                                     wk_v.at[:, 128 * c:128 * (c + 1)], sem_w.at[10 + c])
               for c in range(NT)]
    wcopies = [
        pltpu.make_async_copy(wqkv_hbm.at[:, 0:D], wq_v, sem_w.at[0]),
        pltpu.make_async_copy(wqkv_hbm.at[:, 2 * D:3 * D], wv_v, sem_w.at[1]),
        pltpu.make_async_copy(wo_hbm, wo_v, sem_w.at[2]),
        pltpu.make_async_copy(wg_hbm, wg_v, sem_w.at[3]),
        pltpu.make_async_copy(wu_hbm, wu_v, sem_w.at[4]),
        pltpu.make_async_copy(wd_hbm, wd_v, sem_w.at[5]),
    ]

    def ocopy(r0, n, j):
        return pltpu.make_async_copy(o_v.at[pl.ds(r0, n), :],
                                     o_hbm.at[pl.ds(r0, n), :], sem_o.at[j])

    def tcopy(j):
        c0, c1 = TAILC[j]
        rs = slice(S - TM1 // 2, S)
        return pltpu.make_async_copy(o_v.at[rs, c0:c1], o_hbm.at[rs, c0:c1],
                                     sem_o.at[NB1 + j])

    def perm_lanes(a, tref):
        tref[...] = a.T
        parts = [tref[pl.ds(d, H, stride=DH), :] for d in range(DH)]
        return jnp.concatenate(parts, axis=0).T

    def ln1(i):
        for r in range(i * TM0, (i + 1) * TM0, CH):
            ln_v[r:r + CH, :] = _ln(x_v[r:r + CH, :].astype(f32)).astype(bf16)

    def kphi(i):
        pk = _phi(_dot(ln_v[i * TM0:(i + 1) * TM0, :], wk_v[...]))
        return pk.astype(bf16), jnp.sum(pk, axis=0, keepdims=True)

    def gdot(i, pkb):
        gi = lax.dot_general(pkb, ln_v[i * TM0:(i + 1) * TM0, :],
                             (((0,), (0,)), ((), ())), preferred_element_type=f32)
        if i == 0:
            g_v[...] = gi
        else:
            g_v[...] += gi

    xcopies[0].start()
    for c in kcopies:
        c.start()
    for c in xcopies[1:]:
        c.start()
    for c in wcopies:
        c.start()
    macc_v[...] = jnp.zeros_like(macc_v)
    zq = pl.semaphore_read(z_s)
    xcopies[0].wait()
    ln1(0)
    pks, zs = [], []
    for (c0, c1) in KCH:
        for c in range(c0, c1):
            kcopies[c].wait()
        if c1 == NT:
            xcopies[1].wait()
        pk = _phi(_dot(ln_v[0:TM0, :], wk_v[:, 128 * c0:128 * c1]))
        pks.append(pk.astype(bf16))
        zs.append(jnp.sum(pk, axis=0, keepdims=True))
    pkb = jnp.concatenate(pks, axis=1)
    z = jnp.concatenate(zs, axis=1)

    KS = 512
    for i in range(NB0 - 1):
        gdot(i, pkb)
        ln1(i + 1)
        waits = {1: [xcopies[2]], 3: [xcopies[3]], NB0 - 1: wcopies}.get(i + 1)
        if waits is None:
            pkb, zi = kphi(i + 1)
        else:
            lnb = ln_v[(i + 1) * TM0:(i + 2) * TM0, :]
            ka = _dot(lnb, wk_v[:, 0:KS])
            for c in waits:
                c.wait()
            lnb = ln_v[(i + 1) * TM0:(i + 2) * TM0, :]
            kb = _dot(lnb, wk_v[:, KS:D])
            pk = _phi(jnp.concatenate([ka, kb], axis=1))
            pkb, zi = pk.astype(bf16), jnp.sum(pk, axis=0, keepdims=True)
        z = z + zi

    def prep(c):
        wqp_v[128 * c:128 * (c + 1), :] = perm_lanes(
            wq_v[128 * c:128 * (c + 1), :].astype(f32), t_v).astype(bf16)

    prep(0)
    gdot(NB0 - 1, pkb)

    def qdot(i):
        sl = slice(i * TQ, (i + 1) * TQ)
        pq_v[sl, :] = _phi(_dot(ln_v[sl, :], wqp_v[...]))

    q0 = None
    for c in range(NT):
        if c > 0:
            prep(c)
        part = _dot(ln_v[0:TQ, 128 * c:128 * (c + 1)], wqp_v[128 * c:128 * (c + 1), :])
        q0 = part if q0 is None else q0 + part
    pq_v[0:TQ, :] = _phi(q0)
    zp_v[...] = perm_lanes(jnp.broadcast_to(z, (128, D)), t2_v)[0:8, :]
    kvs = []
    for b, (lo, hi) in enumerate(BAND):
        n = hi - lo
        kvb = _dot(g_v[lo:hi, :].astype(bf16), wv_v[:, 128 * b:128 * (b + 1)])
        rh = (lax.broadcasted_iota(jnp.int32, (n, 128), 0) + lo) // DH
        ch = (lax.broadcasted_iota(jnp.int32, (n, 128), 1) + 128 * b) // DH
        kvs.append(jnp.where(rh == ch, kvb, 0.0).astype(bf16))
    qdot(1)
    for b, (lo, hi) in enumerate(BAND):
        res = _dot(kvs[b], wo_v[128 * b:128 * (b + 1), :])
        for c in range(NT):
            macc_v[c, lo:hi, :] += res[:, 128 * c:128 * (c + 1)]
    qdot(2)
    for c in range(NT):
        for d in range(DH):
            m_v[H * d:H * (d + 1), 128 * c:128 * (c + 1)] = macc_v[
                c, pl.ds(d, H, stride=DH), :].astype(bf16)

    NP = 8
    PR = TM1 // NP

    def gate(ref, tile):
        z0 = pl.multiple_of(zq + S, 8)
        ref[pl.ds(z0, 8), 0:128] = tile

    def norm(r0, p):
        zp = zp_v[0:1, :]
        for rr in range(r0 + p * PR, r0 + (p + 1) * PR, CH):
            pq = pq_v[rr:rr + CH, :]
            t = pq[:, 0:128] * zp[:, 0:128]
            for c in range(1, NT):
                t = t + pq[:, 128 * c:128 * (c + 1)] * zp[:, 128 * c:128 * (c + 1)]
            t = t + pltpu.roll(t, 64, 1)
            t = t + pltpu.roll(t, 32, 1)
            r = 1.0 / (t + 1e-6)
            for c in range(NT):
                pqn_v[rr:rr + CH, 128 * c:128 * (c + 1)] = (
                    pq[:, 128 * c:128 * (c + 1)] * r).astype(bf16)

    def attn(r0):
        h_v[pl.ds(r0, TM1), :] = x_v[pl.ds(r0, TM1), :].astype(f32) + _dot(
            pqn_v[pl.ds(r0, TM1), :], m_v[...])

    def ln2(r0, p):
        for rr in range(r0 + p * PR, r0 + (p + 1) * PR, CH):
            ln2_v[rr:rr + CH, :] = _ln(h_v[rr:rr + CH, :]).astype(bf16)

    FC = 512

    def gsub(r0, c):
        return _dot(ln2_v[pl.ds(r0, TM1), :], wg_v[:, FC * c:FC * (c + 1)])

    def usub(r0, c):
        return _dot(ln2_v[pl.ds(r0, TM1), :], wu_v[:, FC * c:FC * (c + 1)])

    def actst(c, g, u):
        act_v[:, FC * c:FC * (c + 1)] = (jnp.maximum(g, 0.0) * u).astype(bf16)

    def down(r0, lo, n):
        out = h_v[r0 + lo:r0 + lo + n, :] + _dot(act_v[lo:lo + n, :], wd_v[...])
        o_v[r0 + lo:r0 + lo + n, :] = out.astype(bf16)

    def gated(fn, ref, res, r1, p0):
        for t in range(4):
            gate(ref, res[0:8, 128 * t:128 * (t + 1)])
            fn(r1, p0 + t)

    for p in range(NP):
        norm(0, p)
    attn(0)
    qdot(3)
    for p in range(NP):
        ln2(0, p)

    HM = TM1 // 2
    for i in range(NB1):
        r0 = i * TM1
        r1 = (i + 1) * TM1
        nxt = i + 1 < NB1
        g = gsub(r0, 0)
        if nxt:
            gated(norm, pq_v, g, r1, 0)
        u = usub(r0, 0)
        if nxt:
            gated(norm, pq_v, u, r1, 4)
        actst(0, g, u)
        g = gsub(r0, 1)
        u = usub(r0, 1)
        actst(1, g, u)
        if nxt:
            attn(r1)
        g = gsub(r0, 2)
        if nxt:
            gated(ln2, h_v, g, r1, 0)
        u = usub(r0, 2)
        if nxt:
            gated(ln2, h_v, u, r1, 4)
        actst(2, g, u)
        down(r0, 0, HM)
        if not nxt:
            ocopy(r0, HM, NB1 - 1).start()
        if nxt:
            down(r0, HM, HM)
            ocopy(r0, TM1, i).start()
        else:
            for j, (c0, c1) in enumerate(TAILC):
                rs = slice(r0 + HM, r0 + TM1)
                out = h_v[rs, c0:c1] + _dot(act_v[HM:TM1, :], wd_v[:, c0:c1])
                o_v[rs, c0:c1] = out.astype(bf16)
                tcopy(j).start()
    for i in range(NB1 - 1):
        ocopy(i * TM1, TM1, i).wait()
    ocopy(r0, HM, NB1 - 1).wait()
    for j in range(len(TAILC)):
        tcopy(j).wait()


@jax.jit
def pallas_sequential_preLN__linear_attn_block__glu_gated_reglu__prompt_kernel(
    A_x, A_wqkv, A_wo, B_x, B_W_gate, B_W_up, B_W_down,
):
    x = A_x.reshape(S, D)
    anyspec = pl.BlockSpec(memory_space=pl.ANY)
    out = pl.pallas_call(
        _kernel,
        in_specs=[anyspec] * 6,
        out_specs=anyspec,
        out_shape=jax.ShapeDtypeStruct((S, D), bf16),
        scratch_shapes=[
            pltpu.VMEM((S, D), bf16),
            pltpu.VMEM((D, D), bf16),
            pltpu.VMEM((D, D), bf16),
            pltpu.VMEM((D, D), bf16),
            pltpu.VMEM((D, D), bf16),
            pltpu.VMEM((D, F), bf16),
            pltpu.VMEM((D, F), bf16),
            pltpu.VMEM((F, D), bf16),
            pltpu.VMEM((D, D), bf16),
            pltpu.VMEM((S, D), bf16),
            pltpu.VMEM((D, D), f32),
            pltpu.VMEM((NT, D, 128), f32),
            pltpu.VMEM((D, D), bf16),
            pltpu.VMEM((8, D), f32),
            pltpu.VMEM((D, 128), f32),
            pltpu.VMEM((D, 128), f32),
            pltpu.VMEM((S + 8, D), f32),
            pltpu.VMEM((S, D), bf16),
            pltpu.VMEM((S + 8, D), f32),
            pltpu.VMEM((S, D), bf16),
            pltpu.VMEM((S, D), bf16),
            pltpu.VMEM((TM1, F), bf16),
            pltpu.SemaphoreType.REGULAR,
            pltpu.SemaphoreType.DMA((15,)),
            pltpu.SemaphoreType.DMA((NB1 + len(TAILC),)),
        ],
        compiler_params=pltpu.CompilerParams(
            vmem_limit_bytes=100 * 1024 * 1024,
        ),
    )(x, A_wqkv, A_wo, B_W_gate, B_W_up, B_W_down)
    return out.reshape(1, S, D)
```

```python
import jax
import jax.numpy as jnp
from jax import lax
import jax.experimental.pallas as pl
import jax.experimental.pallas.tpu as pltpu

S, D, F, H, DH = 2048, 640, 1536, 32, 20
BLK = [(256 * i, 256 * (i + 1)) for i in range(8)]
XR = [(0, 256), (256, 512), (512, 1024), (1024, 2048)]
WX2, WX3 = 1, 3
NB0 = len(BLK)
TM1 = 256
TQ = 512
NB1 = S // TM1
NT = D // 128
TAILC = [(0, 512), (512, 640)]
CH = 32
KCH = [(0, 2), (2, 4), (4, 5)]
f32 = jnp.float32
bf16 = jnp.bfloat16
BAND = [(0, 144), (120, 264), (240, 400), (376, 520), (496, 640)]


def _ln(x):
    m = jnp.mean(x, axis=-1, keepdims=True)
    xc = x - m
    v = jnp.mean(xc * xc, axis=-1, keepdims=True)
    return xc * lax.rsqrt(v + 1e-5)


def _phi(t):
    return jnp.where(t > 0, t + 1.0, jnp.exp(t)) + 1e-6


def _dot(a, b):
    return jnp.dot(a, b, preferred_element_type=f32)


def _kernel(x_hbm, wqkv_hbm, wo_hbm, wg_hbm, wu_hbm, wd_hbm, o_hbm,
            x_v, wq_v, wk_v, wv_v, wo_v, wg_v, wu_v, wd_v, wqp_v,
            ln_v, g_v, macc_v, m_v, zp_v, t_v, t2_v, pq_v, pqn_v, h_v, ln2_v, o_v, act_v, z_s,
            sem_w, sem_o):
    xcopies = [pltpu.make_async_copy(x_hbm.at[lo:hi, :], x_v.at[lo:hi, :], sem_w.at[6 + j])
               for j, (lo, hi) in enumerate(XR)]
    kcopies = [pltpu.make_async_copy(wqkv_hbm.at[:, D + 128 * c:D + 128 * (c + 1)],
                                     wk_v.at[:, 128 * c:128 * (c + 1)], sem_w.at[10 + c])
               for c in range(NT)]
    wcopies = [
        pltpu.make_async_copy(wqkv_hbm.at[:, 0:D], wq_v, sem_w.at[0]),
        pltpu.make_async_copy(wqkv_hbm.at[:, 2 * D:3 * D], wv_v, sem_w.at[1]),
        pltpu.make_async_copy(wo_hbm, wo_v, sem_w.at[2]),
        pltpu.make_async_copy(wg_hbm, wg_v, sem_w.at[3]),
        pltpu.make_async_copy(wu_hbm, wu_v, sem_w.at[4]),
        pltpu.make_async_copy(wd_hbm, wd_v, sem_w.at[5]),
    ]

    def ocopy(r0, n, j):
        return pltpu.make_async_copy(o_v.at[pl.ds(r0, n), :],
                                     o_hbm.at[pl.ds(r0, n), :], sem_o.at[j])

    def tcopy(j):
        c0, c1 = TAILC[j]
        rs = slice(S - TM1 // 2, S)
        return pltpu.make_async_copy(o_v.at[rs, c0:c1], o_hbm.at[rs, c0:c1],
                                     sem_o.at[NB1 + j])

    def perm_lanes(a, tref):
        tref[...] = a.T
        parts = [tref[pl.ds(d, H, stride=DH), :] for d in range(DH)]
        return jnp.concatenate(parts, axis=0).T

    def ln1(i):
        for r in range(BLK[i][0], BLK[i][1], CH):
            ln_v[r:r + CH, :] = _ln(x_v[r:r + CH, :].astype(f32)).astype(bf16)

    def lnblk(i):
        return ln_v[BLK[i][0]:BLK[i][1], :]

    def kphi(i):
        pk = _phi(_dot(lnblk(i), wk_v[...]))
        return pk.astype(bf16), jnp.sum(pk, axis=0, keepdims=True)

    def gdot(i, pkb):
        gi = lax.dot_general(pkb, lnblk(i),
                             (((0,), (0,)), ((), ())), preferred_element_type=f32)
        if i == 0:
            g_v[...] = gi
        else:
            g_v[...] += gi

    zq = pl.semaphore_read(z_s)
    xcopies[0].start()
    for c in kcopies:
        c.start()
    for c in xcopies[1:]:
        c.start()
    for c in wcopies:
        c.start()
    macc_v[...] = jnp.zeros_like(macc_v)
    xcopies[0].wait()
    ln1(0)
    pks, zs = [], []
    for (c0, c1) in KCH:
        for c in range(c0, c1):
            kcopies[c].wait()
        if c1 == NT:
            xcopies[1].wait()
        pk = _phi(_dot(lnblk(0), wk_v[:, 128 * c0:128 * c1]))
        pks.append(pk.astype(bf16))
        zs.append(jnp.sum(pk, axis=0, keepdims=True))
    pkb = jnp.concatenate(pks, axis=1)
    z = jnp.concatenate(zs, axis=1)

    KS = 512
    for i in range(NB0 - 1):
        gdot(i, pkb)
        ln1(i + 1)
        waits = {WX2: [xcopies[2]], WX3: [xcopies[3]], NB0 - 1: wcopies}.get(i + 1)
        if waits is None:
            pkb, zi = kphi(i + 1)
        else:
            ka = _dot(lnblk(i + 1), wk_v[:, 0:KS])
            for c in waits:
                c.wait()
            kb = _dot(lnblk(i + 1), wk_v[:, KS:D])
            pk = _phi(jnp.concatenate([ka, kb], axis=1))
            pkb, zi = pk.astype(bf16), jnp.sum(pk, axis=0, keepdims=True)
        z = z + zi

    def prep(c):
        wqp_v[128 * c:128 * (c + 1), :] = perm_lanes(
            wq_v[128 * c:128 * (c + 1), :].astype(f32), t_v).astype(bf16)

    prep(0)
    gdot(NB0 - 1, pkb)

    def qdot(i):
        sl = slice(i * TQ, (i + 1) * TQ)
        pq_v[sl, :] = _phi(_dot(ln_v[sl, :], wqp_v[...]))

    q0 = None
    for c in range(NT):
        if c > 0:
            prep(c)
        part = _dot(ln_v[0:TQ, 128 * c:128 * (c + 1)], wqp_v[128 * c:128 * (c + 1), :])
        q0 = part if q0 is None else q0 + part
    pq_v[0:TQ, :] = _phi(q0)
    zp_v[...] = perm_lanes(jnp.broadcast_to(z, (128, D)), t2_v)[0:8, :]
    kvs = []
    for b, (lo, hi) in enumerate(BAND):
        n = hi - lo
        kvb = _dot(g_v[lo:hi, :].astype(bf16), wv_v[:, 128 * b:128 * (b + 1)])
        rh = (lax.broadcasted_iota(jnp.int32, (n, 128), 0) + lo) // DH
        ch = (lax.broadcasted_iota(jnp.int32, (n, 128), 1) + 128 * b) // DH
        kvs.append(jnp.where(rh == ch, kvb, 0.0).astype(bf16))
    qdot(1)
    for b, (lo, hi) in enumerate(BAND):
        res = _dot(kvs[b], wo_v[128 * b:128 * (b + 1), :])
        for c in range(NT):
            macc_v[c, lo:hi, :] += res[:, 128 * c:128 * (c + 1)]
    qdot(2)
    for c in range(NT):
        for d in range(DH):
            m_v[H * d:H * (d + 1), 128 * c:128 * (c + 1)] = macc_v[
                c, pl.ds(d, H, stride=DH), :].astype(bf16)

    NP = 8
    PR = TM1 // NP

    def gate(ref, tile):
        z0 = pl.multiple_of(zq + S, 8)
        ref[pl.ds(z0, 8), 0:128] = tile

    def norm(r0, p):
        zp = zp_v[0:1, :]
        for rr in range(r0 + p * PR, r0 + (p + 1) * PR, CH):
            pq = pq_v[rr:rr + CH, :]
            t = pq[:, 0:128] * zp[:, 0:128]
            for c in range(1, NT):
                t = t + pq[:, 128 * c:128 * (c + 1)] * zp[:, 128 * c:128 * (c + 1)]
            t = t + pltpu.roll(t, 64, 1)
            t = t + pltpu.roll(t, 32, 1)
            r = 1.0 / (t + 1e-6)
            for c in range(NT):
                pqn_v[rr:rr + CH, 128 * c:128 * (c + 1)] = (
                    pq[:, 128 * c:128 * (c + 1)] * r).astype(bf16)

    def attn(r0):
        h_v[pl.ds(r0, TM1), :] = x_v[pl.ds(r0, TM1), :].astype(f32) + _dot(
            pqn_v[pl.ds(r0, TM1), :], m_v[...])

    def ln2(r0, p):
        for rr in range(r0 + p * PR, r0 + (p + 1) * PR, CH):
            ln2_v[rr:rr + CH, :] = _ln(h_v[rr:rr + CH, :]).astype(bf16)

    FC = 512

    def gsub(r0, c):
        return _dot(ln2_v[pl.ds(r0, TM1), :], wg_v[:, FC * c:FC * (c + 1)])

    def usub(r0, c):
        return _dot(ln2_v[pl.ds(r0, TM1), :], wu_v[:, FC * c:FC * (c + 1)])

    def actst(c, g, u):
        act_v[:, FC * c:FC * (c + 1)] = (jnp.maximum(g, 0.0) * u).astype(bf16)

    def down(r0, lo, n):
        out = h_v[r0 + lo:r0 + lo + n, :] + _dot(act_v[lo:lo + n, :], wd_v[...])
        o_v[r0 + lo:r0 + lo + n, :] = out.astype(bf16)

    def gated(fn, ref, res, r1, p0):
        for t in range(4):
            gate(ref, res[0:8, 128 * t:128 * (t + 1)])
            fn(r1, p0 + t)

    for p in range(NP):
        norm(0, p)
    attn(0)
    qdot(3)
    for p in range(NP):
        ln2(0, p)

    HM = TM1 // 2
    for i in range(NB1):
        r0 = i * TM1
        r1 = (i + 1) * TM1
        nxt = i + 1 < NB1
        g = gsub(r0, 0)
        if nxt:
            gated(norm, pq_v, g, r1, 0)
        u = usub(r0, 0)
        if nxt:
            gated(norm, pq_v, u, r1, 4)
        actst(0, g, u)
        g = gsub(r0, 1)
        u = usub(r0, 1)
        actst(1, g, u)
        if nxt:
            attn(r1)
        g = gsub(r0, 2)
        if nxt:
            gated(ln2, h_v, g, r1, 0)
        u = usub(r0, 2)
        if nxt:
            gated(ln2, h_v, u, r1, 4)
        actst(2, g, u)
        down(r0, 0, HM)
        if not nxt:
            ocopy(r0, HM, NB1 - 1).start()
        if nxt:
            down(r0, HM, HM)
            ocopy(r0, TM1, i).start()
        else:
            for j, (c0, c1) in enumerate(TAILC):
                rs = slice(r0 + HM, r0 + TM1)
                out = h_v[rs, c0:c1] + _dot(act_v[HM:TM1, :], wd_v[:, c0:c1])
                o_v[rs, c0:c1] = out.astype(bf16)
                tcopy(j).start()
    for i in range(NB1 - 1):
        ocopy(i * TM1, TM1, i).wait()
    ocopy(r0, HM, NB1 - 1).wait()
    for j in range(len(TAILC)):
        tcopy(j).wait()


@jax.jit
def pallas_sequential_preLN__linear_attn_block__glu_gated_reglu__prompt_kernel(
    A_x, A_wqkv, A_wo, B_x, B_W_gate, B_W_up, B_W_down,
):
    x = A_x.reshape(S, D)
    anyspec = pl.BlockSpec(memory_space=pl.ANY)
    out = pl.pallas_call(
        _kernel,
        in_specs=[anyspec] * 6,
        out_specs=anyspec,
        out_shape=jax.ShapeDtypeStruct((S, D), bf16),
        scratch_shapes=[
            pltpu.VMEM((S, D), bf16),
            pltpu.VMEM((D, D), bf16),
            pltpu.VMEM((D, D), bf16),
            pltpu.VMEM((D, D), bf16),
            pltpu.VMEM((D, D), bf16),
            pltpu.VMEM((D, F), bf16),
            pltpu.VMEM((D, F), bf16),
            pltpu.VMEM((F, D), bf16),
            pltpu.VMEM((D, D), bf16),
            pltpu.VMEM((S, D), bf16),
            pltpu.VMEM((D, D), f32),
            pltpu.VMEM((NT, D, 128), f32),
            pltpu.VMEM((D, D), bf16),
            pltpu.VMEM((8, D), f32),
            pltpu.VMEM((D, 128), f32),
            pltpu.VMEM((D, 128), f32),
            pltpu.VMEM((S + 8, D), f32),
            pltpu.VMEM((S, D), bf16),
            pltpu.VMEM((S + 8, D), f32),
            pltpu.VMEM((S, D), bf16),
            pltpu.VMEM((S, D), bf16),
            pltpu.VMEM((TM1, F), bf16),
            pltpu.SemaphoreType.REGULAR,
            pltpu.SemaphoreType.DMA((15,)),
            pltpu.SemaphoreType.DMA((NB1 + len(TAILC),)),
        ],
        compiler_params=pltpu.CompilerParams(
            vmem_limit_bytes=100 * 1024 * 1024,
        ),
    )(x, A_wqkv, A_wo, B_W_gate, B_W_up, B_W_down)
    return out.reshape(1, S, D)
```
